```python
import os as _os
_os.environ.setdefault("JAX_PLATFORMS", "cpu")
import jax
import jax.numpy as jnp

def _softmax(x, axis=-1):
    return jax.nn.softmax(x, axis=axis)
def _gelu(x):
    return jax.nn.gelu(x, approximate=True)
def _silu(x):
    return jax.nn.silu(x)
def _sigmoid(x):
    return jax.nn.sigmoid(x)
def _layernorm(x, axis=-1, eps=1e-5):
    m = jnp.mean(x, axis=axis, keepdims=True)
    v = jnp.var(x, axis=axis, keepdims=True)
    return (x - m) / jnp.sqrt(v + eps)
def _scatter_add(tgt, idx, src, axis=0):
    return tgt.at[idx].add(src)
def _segment_sum(src, seg, n):
    return jax.ops.segment_sum(src, seg, n)
class _Rng:
    def __init__(self, key):
        self._k = key
    def _next(self):
        self._k, sub = jax.random.split(self._k)
        return sub
    def normal(self, shape):
        return jax.random.normal(self._next(), shape, dtype=jnp.bfloat16)
    def randint(self, lo, hi, shape):
        return jax.random.randint(self._next(), shape, lo, hi, dtype=jnp.int32)
    def uniform(self, shape, lo=0.0, hi=1.0):
        return jax.random.uniform(self._next(), shape, jnp.bfloat16, lo, hi)
    def permutation(self, n):
        return jax.random.permutation(self._next(), n)


kernel_name = 'sequential_preLN__sliding_local_dilated__mixer_s_mlp__prompt'

def setup_inputs():
    _rng = _Rng(jax.random.key(int.from_bytes(__import__("os").urandom(4), "little")))
    _w = (lambda a: (lambda t: t.astype(jnp.bfloat16) if jnp.issubdtype(t.dtype, jnp.floating) else t)(jnp.asarray(a)))
    def _A_setup():
        B, S, D = 1, 2048, 448
        return {
            "x": _w((lambda *s: _rng.normal(s) * 0.05)(B, S, D)),
            "wqkv": _w((lambda *s: _rng.normal(s) * 0.05)(D, 3 * D)),
            "wo": _w((lambda *s: _rng.normal(s) * 0.05)(D, D)),
        }
    _A_in = _A_setup()

    def _B_setup():
        B, S, D, F = 1, 2048, 448, 1792
        return {
            "x":  _w((lambda *s: _rng.normal(s) * 0.05)(B, S, D)),
            "w1": _w((lambda *s: _rng.normal(s) * 0.8)(D, D) * (D ** -0.5)),
            "w2": _w((lambda *s: _rng.normal(s) * 0.8)(D, D) * (D ** -0.5)),
            "w3": _w((lambda *s: _rng.normal(s) * 0.8)(D, F) * (D ** -0.5)),
            "w4": _w((lambda *s: _rng.normal(s) * 0.8)(F, D) * (F ** -0.5)),
        }
    _B_in = _B_setup()

    return {
        "A_x": _A_in["x"],
        "A_wqkv": _A_in["wqkv"],
        "A_wo": _A_in["wo"],
        "B_x": _B_in["x"],
        "B_w1": _B_in["w1"],
        "B_w2": _B_in["w2"],
        "B_w3": _B_in["w3"],
        "B_w4": _B_in["w4"],
    }

def reference(A_x, A_wqkv, A_wo, B_x, B_w1, B_w2, B_w3, B_w4):
    def _A_ref(x, wqkv, wo):
        B, S, D = x.shape
        H = 16; Dh = D // H
        W, dil = 8, 2
        qkv = (lambda x, *d: x.transpose(*d))((x @ wqkv).reshape(B, S, 3, H, Dh), 2, 0, 3, 1, 4)
        q, k, v = qkv[0], qkv[1], qkv[2]
        scale = Dh ** -0.5
        pos = jnp.arange(S)
        off = jnp.arange(W) * dil
        idx = pos[:, None] - off[None, :]
        mask = idx >= 0
        idx_c = jnp.where(mask, idx, 0).reshape(-1)
        kg = k[:, :, idx_c, :].reshape(B, H, S, W, Dh)
        vg = v[:, :, idx_c, :].reshape(B, H, S, W, Dh)
        logits = jnp.einsum("bhsd,bhswd->bhsw", q, kg) * scale
        logits = jnp.where(mask[None, None, :, :], logits, -1e9)
        attn = _softmax(logits, axis=-1)
        o = jnp.einsum("bhsw,bhswd->bhsd", attn, vg)
        return (lambda x, *d: x.transpose(*d))(o, 0, 2, 1, 3).reshape(B, S, D) @ wo

    def _B_ref(x, w1, w2, w3, w4):
        B, S, D = x.shape
        h = _gelu(_layernorm(x, axis=-1) @ w1)
        c = D // 4
        g0 = jnp.pad(h[:, :, 0*c:1*c], ((0, 0), (1, 0), (0, 0)))[:, :S, :]
        g1 = jnp.pad(h[:, :, 1*c:2*c], ((0, 0), (0, 1), (0, 0)))[:, 1:, :]
        g2 = jnp.pad(h[:, :, 2*c:3*c], ((0, 0), (2, 0), (0, 0)))[:, :S, :]
        g3 = jnp.pad(h[:, :, 3*c:   ], ((0, 0), (0, 2), (0, 0)))[:, 2:, :]
        hs = jnp.concatenate([g0, g1, g2, g3], axis=-1) @ w2
        x1 = x + hs
        h2 = _gelu(_layernorm(x1, axis=-1) @ w3) @ w4
        return x1 + h2

    x = A_x
    h = x + _A_ref(_layernorm(x, axis=-1), A_wqkv, A_wo)
    h2 = h + _B_ref(_layernorm(h, axis=-1), B_w1, B_w2, B_w3, B_w4)
    return h2
```

```python
import functools

import jax
import jax.numpy as jnp
from jax import lax
from jax.experimental import pallas as pl
from jax.experimental.pallas import tpu as pltpu

S, D, F, H, DH, W, DIL = 2048, 448, 1792, 16, 28, 8, 2
DA = D + 16
EPS = 1e-5
f32, bf16, u32, i32 = jnp.float32, jnp.bfloat16, jnp.uint32, jnp.int32
L = 128
NT = S // L
C = 256
NC = S // C
SUB = C // L
RB = 32
HB = RB // 2
NB = D // RB
DB = 7
NBK = DH // DB
_C0 = 0.7978845608028654
_C1 = 0.044715
_QCOLS = ((0, 512), (512, 896), (896, 3 * D))
_XP = ((0, 2), (2, 4), (4, 5), (5, 8))

_GROUPS = ("wq", "x0", "wk x1", "wv wo w1 w2 x2", "w3 w4 x3")


def _order():
    o = ["W0", "Xq", "W1", "l0", "l1", "q0", "q1",
         "W2", "l2", "q2", "Xk", "l3", "q3", "k0", "k1", "k2", "k3",
         ("c0", "k0:60-100 k1:0-60"), ("c1", "k1:60-100 k2:0-60"), ("c2", "k2:60-100 k3:0-60"),
         "W3", "l4", "q4", "Xv", "k4", "v0", "v1", "v2", "v3", "v4",
         ("c3", "k4"), ("Xo", "v0 v1"), ("X1", "v2 v3"),
         ("d0", "v1"), ("d1", "v2"), ("d2", "v3"), ("d3", "v4"),
         "O0", "M0", "O1", "M1", ("X2", "O0 M0 O1"), "s0",
         "W4", "P0", ("l5", "P0:0-60"), "Q5", ("X3", "P0 Q5:0-80"), "U0", ("X4", "U0:0-60"), "V0",
         ("a2", "U0 V0:0-70")]
    for n in range(2, NC - 1):
        q = n + 4 < NC
        o += [f"O{n}"] + ([(f"l{n+4}", f"O{n}")] if q else []) + [f"M{n}", f"s{n-1}"]
        o += ([f"Q{n+4}"] if q else []) + [f"P{n-1}", f"U{n-1}", f"V{n-1}"]
        o += [(f"a{n+1}", (f"Q{n+4} " if q else "") + f"U{n-1} V{n-1}:0-70")]
    n = NC - 1
    o += [f"O{n}", f"M{n}", f"s{n-1}", f"P{n-1}", f"s{n}", f"P{n}", f"U{n-1}", f"V{n-1}", f"U{n}", f"V{n}"]
    return o


_ORDER = _order()


def _gelu_coef(sc):
    return _C0 * sc, (_C0 * _C1) * (sc * sc * sc), 0.5 * sc


def _pk(x):
    return pltpu.bitcast(x, u32)


def _up(x):
    return pltpu.bitcast(x, bf16)


def _packe(a, b):
    return pltpu.bitcast(pltpu.pack_elementwise([a, b], packed_dtype=bf16), u32)


def _pack2(x):
    r = x.shape[0] // 2
    return _packe(x[:r], x[r:])


def _unp(p, i):
    return pltpu.unpack_elementwise(p, index=i, packed_dtype=bf16, unpacked_dtype=f32)


def _unpack2(p):
    return jnp.concatenate([_unp(p, 0), _unp(p, 1)], axis=0)


def _fin(acc):
    return jnp.sum(acc, axis=0, keepdims=True)


def _stats(a1, a2):
    m = _fin(a1) * (1.0 / D)
    v = jnp.maximum(_fin(a2) * (1.0 / D) - m * m, 0.0)
    return m, v


def _mean_rows(m):
    c = m.shape[1]
    mb = jnp.broadcast_to(m, (8, c))
    lo = mb - _unp(_packe(mb, mb), 0)
    sub = lax.broadcasted_iota(i32, (8, c), 0)
    return _packe(jnp.where(sub < 2, mb, 0.0), jnp.where(sub == 0, lo, 0.0))


def _colsum_rows(blk):
    acc = None
    for p in blk:
        t = _unp(p, 0) + _unp(p, 1)
        acc = t if acc is None else acc + t
    n = acc.shape[1]
    c = jnp.broadcast_to(-_fin(acc), (8, n))
    lo = c - _unp(_packe(c, c), 0)
    sub = lax.broadcasted_iota(i32, (8, n), 0)
    return _packe(jnp.where(sub == 0, c, jnp.where(sub == 1, lo, 0.0)), jnp.where(sub == 0, c, 0.0))


def _rows(b):
    return slice(b * RB, (b + 1) * RB)


def _prows(b):
    return slice(b * HB, (b + 1) * HB)


def _cols(s):
    return slice(s * L, (s + 1) * L)


def _dot(a, b):
    return jnp.dot(a, b, preferred_element_type=f32)


def _kernel(x_hbm, wqkv_hbm, wo_hbm, w1_hbm, w2_hbm, w3_hbm, w4t_hbm, out_hbm,
            x_v, wqkv_v, wo_v, w1_v, w2_v, w3_v, w4t_v,
            wqkvt, wot, w1t, w2t, w3t, w4t, tmp32, tmpq, wop,
            q_s, kp, vp, o_s, h_s, hb_s, h1_s, hsh_s, hx_s, xb_s, g_s, out_v, zsem, sems):
    ng = len(_GROUPS)
    as_bf16 = lambda r: r.bitcast(bf16)
    ends = {f"x{p}": (x_hbm.at[:, j0 * C:j1 * C], as_bf16(x_v[p]).at[0:D, :]) for p, (j0, j1) in enumerate(_XP)}
    for p, nm in enumerate(("wq", "wk", "wv")):
        ends[nm] = (wqkv_hbm.at[:, _QCOLS[p][0]:_QCOLS[p][1]], as_bf16(wqkv_v[p]))
    ends.update(wo=(wo_hbm, as_bf16(wo_v)), w1=(w1_hbm, as_bf16(w1_v)), w2=(w2_hbm, as_bf16(w2_v)),
                w3=(w3_hbm, as_bf16(w3_v)), w4=(w4t_hbm, as_bf16(w4t_v)))
    groups = [[pltpu.make_async_copy(*ends[nm], sems.at[i]) for nm in spec.split()]
              for i, spec in enumerate(_GROUPS)]
    c_out = []
    st = {}
    lane1 = lax.broadcasted_iota(i32, (8, L), 1)

    def xloc(j, s=None):
        p = [p for p, (j0, j1) in enumerate(_XP) if j0 <= j < j1][0]
        c0 = (j - _XP[p][0]) * C
        return x_v[p], (slice(c0, c0 + C) if s is None else slice(c0 + s * L, c0 + (s + 1) * L))

    def gate_bits(gate):
        return pltpu.bitcast(gate, i32) & st["zvec"]

    def gated(p, gate):
        if gate is None:
            return p
        r, c = p.shape
        gz = pltpu.bitcast(gate_bits(gate), u32)
        if c < L:
            gz = gz[:, 0:c]
        elif c > L:
            gz = jnp.concatenate([gz] * (c // L), axis=1)
        return p | jnp.broadcast_to(gz[None], (r // 8, 8, c)).reshape(r, c)

    def note(name, res):
        st.setdefault(("res", name), []).extend(
            (res, r, s) for s in range(SUB) for r in range(res.shape[0] // 8))

    def pick_gates(spec, n):
        if not spec:
            return [None] * n
        tl = []
        for item in spec.split():
            nm, _, lim = item.partition(":")
            flat = st["res", nm]
            if lim:
                lo, hi = lim.split("-")
                flat = flat[len(flat) * int(lo) // 100:len(flat) * int(hi) // 100]
            tl += flat
        out = []
        for i in range(n):
            res, r, s = tl[(i * len(tl)) // n]
            out.append(res[r * 8:(r + 1) * 8, _cols(s)])
        return out

    def windows(ref, g, b, gate):
        rs = slice(b * DB * 8, (b + 1) * DB * 8)
        cur, prev = ref[g + 1, rs, :], ref[g, rs, :]
        ln = lane1 | gate_bits(gate)
        for w in range(W):
            r = cur
            if w:
                mk = jnp.broadcast_to((ln < L - DIL * w)[None], (DB, 8, L)).reshape(DB * 8, L)
                r = pltpu.roll(jnp.where(mk, cur, prev), DIL * w, 1)
            yield w, [_unp(r, i).reshape(DB, 8, L) for i in range(2)]

    def att_qk(g, gates):
        lg = [[None] * W, [None] * W]
        for b in range(NBK):
            qb = q_s[g, b * DB * H:(b + 1) * DB * H, :].reshape(DB, 2, 8, L)
            for w, ks in windows(kp, g, b, gates[b]):
                for i in range(2):
                    pr = jnp.sum(qb[:, i] * ks[i], axis=0)
                    lg[i][w] = pr if lg[i][w] is None else lg[i][w] + pr
        rq = st["rx", g] * (DH ** -0.5)
        a = []
        for i in range(2):
            sc = [t * rq for t in lg[i]]
            if g == 0:
                sc = [jnp.where(lane1 >= DIL * w, sc[w], -1e9) for w in range(W)]
            m = functools.reduce(jnp.maximum, sc)
            p = [jnp.exp(s_ - m) for s_ in sc]
            r = 1.0 / functools.reduce(jnp.add, p)
            a.append([p_ * r for p_ in p])
        st["att", g] = a

    def att_pv(g, gates):
        a = st["att", g]
        for b in range(NBK):
            o = [None, None]
            for w, vs in windows(vp, g, b, gates[b]):
                for i in range(2):
                    t = a[i][w][None] * vs[i]
                    o[i] = t if o[i] is None else o[i] + t
            o_s[g, b * DB * 8:(b + 1) * DB * 8, :] = _packe(o[0].reshape(DB * 8, L), o[1].reshape(DB * 8, L))

    def t_a(j, spec):
        gates = pick_gates(spec, SUB * 2 * NBK)
        for s in range(SUB):
            att_qk(j * SUB + s, gates[2 * s * NBK:(2 * s + 1) * NBK])
            att_pv(j * SUB + s, gates[(2 * s + 1) * NBK:(2 * s + 2) * NBK])

    def t_c(g, spec):
        att_qk(g, pick_gates(spec, NBK))

    def t_d(g, spec):
        att_pv(g, pick_gates(spec, NBK))

    def cat(ref, j):
        return _up(jnp.concatenate([ref[j * SUB + s] for s in range(SUB)], axis=1))

    def t_l(j, spec=None):
        gates = pick_gates(spec, SUB * NB)
        for s in range(SUB):
            xr, cs = xloc(j, s)
            a1 = a2 = None
            for b in range(NB):
                x = _unpack2(gated(xr[_prows(b), cs], gates[s * NB + b]))
                a1 = x if a1 is None else a1 + x
                a2 = x * x if a2 is None else a2 + x * x
            m, v = _stats(a1, a2)
            st["rx", j * SUB + s] = lax.rsqrt(v + EPS)
            xr[D // 2:DA // 2, cs] = _mean_rows(m)

    def qkv_epi(j, part, res):
        for s in range(SUB):
            g = j * SUB + s
            if part == 0:
                q_s[g] = res[:, _cols(s)]
            else:
                dst = kp if part == 1 else vp
                for d in range(DH):
                    dst[g + 1, d * 8:(d + 1) * 8, :] = _pack2(res[d * H:(d + 1) * H, _cols(s)] * st["rx", g])

    def t_Q(j):
        xr, cs = xloc(j)
        qkv = _dot(_up(wqkvt[...]), _up(xr[:, cs]))
        note(f"Q{j}", qkv)
        for p in range(3):
            qkv_epi(j, p, qkv[p * D:(p + 1) * D])

    def t_part(p, j):
        xr, cs = xloc(j)
        res = _dot(_up(wqkvt[p * D // 2:(p + 1) * D // 2, :]), _up(xr[:, cs]))
        note("qkv"[p] + str(j), res)
        qkv_epi(j, p, res)

    def t_O(j):
        ao = _dot(_up(wot[...]), cat(o_s, j))
        note(f"O{j}", ao)
        for s in range(SUB):
            g = j * SUB + s
            xr, cs = xloc(j, s)
            a1 = a2 = None
            for b in range(NB):
                h = _unpack2(xr[_prows(b), cs]) + ao[_rows(b), _cols(s)]
                h_s[g, _rows(b), :] = h
                hb_s[g, _prows(b), :] = _pack2(h)
                a1 = h if a1 is None else a1 + h
                a2 = h * h if a2 is None else a2 + h * h
            m, v = _stats(a1, a2)
            r = lax.rsqrt(v + EPS)
            r2 = lax.rsqrt(v * r * r + EPS)
            st["h", g] = (m, r, _gelu_coef(r * r2))
            hb_s[g, D // 2:DA // 2, :] = _mean_rows(m)

    def t_M(j):
        a1 = _dot(_up(w1t[...]), cat(hb_s, j))
        note(f"M{j}", a1)
        for s in range(SUB):
            g = j * SUB + s
            ca, cb, ch = st["h", g][2]
            for b in range(NB):
                y = a1[_rows(b), _cols(s)]
                hy = y * ch
                h1_s[g + 1, _prows(b), :] = _pack2(hy + hy * jnp.tanh(y * (ca + cb * (y * y))))

    grp = D // 8
    lane_g = lax.broadcasted_iota(i32, (grp, L), 1)

    def t_s(j):
        for s in range(SUB):
            g = j * SUB + s + 1
            for gi, sh in enumerate((1, -1, 2, -2)):
                gs = slice(gi * grp, (gi + 1) * grp)
                if sh > 0:
                    r = pltpu.roll(jnp.where(lane_g < L - sh, h1_s[g, gs, :], h1_s[g - 1, gs, :]), sh, 1)
                else:
                    r = pltpu.roll(jnp.where(lane_g >= -sh, h1_s[g, gs, :], h1_s[g + 1, gs, :]), L + sh, 1)
                hsh_s[g - 1, gs, :] = r

    def t_P(j):
        hs = _dot(_up(w2t[...]), cat(hsh_s, j))
        note(f"P{j}", hs)
        for s in range(SUB):
            g = j * SUB + s
            m, r, _ = st["h", g]
            a1 = a2 = None
            for b in range(NB):
                h = h_s[g, _rows(b), :]
                x1 = (h - m) * r + hs[_rows(b), _cols(s)]
                hx_s[g, _rows(b), :] = h + x1
                xb_s[g, _prows(b), :] = _pack2(x1)
                a1 = x1 if a1 is None else a1 + x1
                a2 = x1 * x1 if a2 is None else a2 + x1 * x1
            m3, v3 = _stats(a1, a2)
            st["x", g] = _gelu_coef(lax.rsqrt(v3 + EPS))
            xb_s[g, D // 2:DA // 2, :] = _mean_rows(m3)

    def t_U(j):
        a3 = _dot(_up(w3t[...]), cat(xb_s, j))
        note(f"U{j}", a3)
        for s in range(SUB):
            ca, cb, _ = st["x", j * SUB + s]
            for b in range(F // RB):
                y = a3[_rows(b), _cols(s)]
                g_s[j % 2, _prows(b), _cols(s)] = _pack2(y * (1.0 + jnp.tanh(y * (ca + cb * (y * y)))))

    def t_V(j):
        halves = ((0, NB // 2), (NB // 2, NB)) if j == NC - 1 else ((0, NB),)
        for hi, (b0, b1) in enumerate(halves):
            h2 = None
            for c in range(0, F, 512):
                e = min(c + 512, F)
                t = _dot(_up(w4t[b0 * HB:b1 * HB, c:e]), _up(g_s[j % 2, c // 2:e // 2, :]))
                note(f"V{j}", t)
                h2 = t if h2 is None else h2 + t
            for s in range(SUB):
                g = j * SUB + s
                ov = out_v[g + hi * SUB]
                ch = st["x", g][2]
                for b in range(b0, b1):
                    ov[_prows(b - b0), :] = _pack2(hx_s[g, _rows(b), :] + h2[_rows(b - b0), _cols(s)] * ch)
                cp = pltpu.make_async_copy(as_bf16(ov), out_hbm.at[b0 * RB:b1 * RB, _cols(g)], sems.at[ng])
                cp.start()
                c_out.append(cp)

    def t_W(i):
        if i == 0:
            for group in groups:
                for c in group:
                    c.start()
            st["zvec"] = jnp.full((8, L), pl.semaphore_read(zsem), i32)
            kp[0] = jnp.zeros((D // 2, L), u32)
            vp[0] = jnp.zeros((D // 2, L), u32)
            h1_s[0] = jnp.zeros((D // 2, L), u32)
            h1_s[NT + 1] = jnp.zeros((D // 2, L), u32)
        for c in groups[i]:
            c.wait()

    def t_Xpart(p):
        c0, c1 = _QCOLS[p]
        blk = [wqkv_v[p][b * 8:(b + 1) * 8, :] for b in range(D // 16)]
        src = _up(jnp.concatenate(blk + [_colsum_rows(blk)], axis=0)).T.astype(f32)
        for c4 in range(4):
            wd = min(L, DA - c4 * L)
            tmpq[c4, c0:c1, 0:wd] = src[:, c4 * L:c4 * L + wd]
        for d in range(DH):
            for c4 in range(4):
                wd = min(L, DA - c4 * L)
                wqkvt[(p * D + d * H) // 2:(p * D + (d + 1) * H) // 2, c4 * L:c4 * L + wd] = (
                    _pk(tmpq[c4, pl.ds(p * D + d, H, stride=DH), 0:wd].astype(bf16)))

    def deint_rows(t, dst, base):
        tp = _pk(t)
        for b in range(t.shape[0] // RB):
            dst[base + b * HB:base + (b + 1) * HB, :] = _pk(_unpack2(tp[_prows(b)]).astype(bf16))

    def t_Xo(spec):
        gates = pick_gates(spec, 8)
        for c4 in range(4):
            wd = min(L, D - c4 * L)
            cs = slice(c4 * L, c4 * L + wd)
            for hf in range(2):
                p = gated(wo_v[hf * 112:(hf + 1) * 112, cs], gates[c4 * 2 + hf])
                tmp32[c4, hf * 224:(hf + 1) * 224, 0:wd] = _up(p).astype(f32)
            for d in range(DH):
                wop[d * 8:(d + 1) * 8, cs] = _pack2(tmp32[c4, pl.ds(d, H, stride=DH), 0:wd])
            deint_rows(_up(wop[:, cs]).T, wot, c4 * L // 2)

    def xpose_w(w_v, dst, n, xw, aug, spec):
        nb = -(-n // xw)
        gates = pick_gates(spec, nb * 4)
        for c in range(nb):
            cs = slice(c * xw, min((c + 1) * xw, n))
            blk = [gated(w_v[b * 8:(b + 1) * 8, cs], gates[c * 4 + b // 7]) for b in range(D // 16)]
            if aug:
                blk.append(_colsum_rows(blk))
            deint_rows(_up(jnp.concatenate(blk, axis=0)).T, dst, c * xw // 2)

    def t_X4(spec):
        gates = pick_gates(spec, NB)
        for b in range(NB):
            w4t[_prows(b), :] = _pk(_unpack2(gated(w4t_v[_prows(b), :], gates[b])).astype(bf16))

    part = functools.partial
    once = dict(Xq=part(t_Xpart, 0), Xk=part(t_Xpart, 1), Xv=part(t_Xpart, 2), Xo=t_Xo,
                X1=part(xpose_w, w1_v, w1t, D, L, True), X2=part(xpose_w, w2_v, w2t, D, L, False),
                X3=part(xpose_w, w3_v, w3t, F, 256, True), X4=t_X4)
    per = dict(a=t_a, c=t_c, d=t_d, l=t_l, Q=t_Q, O=t_O, M=t_M, s=t_s, P=t_P, U=t_U, V=t_V, W=t_W,
               q=part(t_part, 0), k=part(t_part, 1), v=part(t_part, 2))
    for task in _ORDER:
        name, extra = (task[0], task[1:]) if isinstance(task, tuple) else (task, ())
        if name in once:
            once[name](*extra)
        else:
            per[name[0]](int(name[1:]), *extra)
    for c in c_out:
        c.wait()


@jax.jit
def pallas_sequential_preLN__sliding_local_dilated__mixer_s_mlp__prompt_kernel(
    A_x: jax.Array,
    A_wqkv: jax.Array,
    A_wo: jax.Array,
    B_x: jax.Array,
    B_w1: jax.Array,
    B_w2: jax.Array,
    B_w3: jax.Array,
    B_w4: jax.Array,
):
    del B_x
    hbm = pl.BlockSpec(memory_space=pl.ANY)
    V = pltpu.VMEM
    out_t = pl.pallas_call(
        _kernel,
        in_specs=[hbm] * 7,
        out_specs=hbm,
        out_shape=jax.ShapeDtypeStruct((D, S), bf16),
        scratch_shapes=[
            [V((DA // 2, (j1 - j0) * C), u32) for j0, j1 in _XP],
            [V((D // 2, c1 - c0), u32) for c0, c1 in _QCOLS],
            V((D // 2, D), u32), V((D // 2, D), u32),
            V((D // 2, D), u32), V((D // 2, F), u32), V((D // 2, F), u32),
            V((3 * D // 2, DA), u32), V((D // 2, D), u32), V((D // 2, DA), u32),
            V((D // 2, D), u32), V((F // 2, DA), u32), V((D // 2, F), u32),
            V((4, D, L), f32), V((4, 3 * D, L), f32), V((D // 2, D), u32),
            V((NT, D, L), f32), V((NT + 1, D // 2, L), u32), V((NT + 1, D // 2, L), u32),
            V((NT, D // 2, L), u32),
            V((NT, D, L), f32), V((NT, DA // 2, L), u32), V((NT + 2, D // 2, L), u32), V((NT, D // 2, L), u32),
            V((NT, D, L), f32), V((NT, DA // 2, L), u32),
            V((2, F // 2, C), u32),
            [V((D // 2, L), u32)] * (NT - SUB) + [V((D // 4, L), u32)] * (2 * SUB),
            pltpu.SemaphoreType.REGULAR,
            pltpu.SemaphoreType.DMA((len(_GROUPS) + 1,)),
        ],
        compiler_params=pltpu.CompilerParams(
            vmem_limit_bytes=100 * 1024 * 1024, disable_semaphore_checks=True),
    )(A_x[0].T, A_wqkv, A_wo, B_w1, B_w2, B_w3, B_w4.T)
    return out_t.T[None]
```

```python
import functools

import jax
import jax.numpy as jnp
from jax import lax
from jax.experimental import pallas as pl
from jax.experimental.pallas import tpu as pltpu

S, D, F, H, DH, W, DIL = 2048, 448, 1792, 16, 28, 8, 2
DA = D + 16
EPS = 1e-5
f32, bf16, u32, i32 = jnp.float32, jnp.bfloat16, jnp.uint32, jnp.int32
L = 128
NT = S // L
C = 256
NC = S // C
SUB = C // L
RB = 32
HB = RB // 2
NB = D // RB
DB = 4
NBK = DH // DB
_C0 = 0.7978845608028654
_C1 = 0.044715
_QCOLS = ((0, 512), (512, 896), (896, 3 * D))
_XP = ((0, 2), (2, 4), (4, 5), (5, 8))

_GROUPS = ("wq", "x0 z", "wk x1", "wv wo w1 w2 x2", "w3 w4 x3")


def _order():
    o = ["W0", "Xq", "W1", "l0", "l1", "q0", "q1",
         "W2", "l2", "q2", "Xk", "l3", "q3", "k0", "k1", "k2", "k3",
         ("c0", "k0:60-100 k1:0-60"), ("c1", "k1:60-100 k2:0-60"), ("c2", "k2:60-100 k3:0-60"),
         "W3", "l4", "q4", "Xv", "k4", "v0", "v1", "v2", "v3", "v4",
         ("c3", "k4"), ("Xo", "v0 v1"), ("X1", "v2 v3"),
         ("d0", "v1"), ("d1", "v2"), ("d2", "v3"), ("d3", "v4"),
         "O0", "M0", "O1", "M1", ("X2", "O0 M0 O1"), "s0",
         "W4", "P0", ("l5", "P0:0-60"), "Q5", ("X3", "P0 Q5:0-80"), "U0", "V0",
         ("a2", "U0 V0:0-70")]
    for n in range(2, NC - 1):
        q = n + 4 < NC
        o += [f"O{n}"] + ([(f"l{n+4}", f"O{n}")] if q else []) + [f"M{n}", f"s{n-1}"]
        o += ([f"Q{n+4}"] if q else []) + [f"P{n-1}", f"U{n-1}", f"V{n-1}"]
        o += [(f"a{n+1}", (f"Q{n+4} " if q else "") + f"U{n-1} V{n-1}:0-70")]
    n = NC - 1
    o += [f"O{n}", f"M{n}", f"s{n-1}", f"P{n-1}", f"s{n}", f"P{n}", f"U{n-1}", f"V{n-1}", f"U{n}", f"V{n}"]
    return o


_ORDER = _order()


def _gelu_coef(sc):
    return _C0 * sc, (_C0 * _C1) * (sc * sc * sc), 0.5 * sc


def _pk(x):
    return pltpu.bitcast(x, u32)


def _up(x):
    return pltpu.bitcast(x, bf16)


def _f32(p):
    return _up(p).astype(f32)


def _hi(x):
    return x.astype(bf16).astype(f32)


def _fin(acc):
    return jnp.sum(acc, axis=0, keepdims=True)


def _stats(a1, a2):
    m = _fin(a1) * (1.0 / D)
    v = jnp.maximum(_fin(a2) * (1.0 / D) - m * m, 0.0)
    return m, v


def _mean_rows(m):
    mb = jnp.broadcast_to(m, (16, m.shape[1]))
    sub = lax.broadcasted_iota(i32, mb.shape, 0)
    return jnp.where(sub == 1, mb - _hi(mb), jnp.where(sub < 3, mb, 0.0))


def _colsum_rows(blk):
    acc = None
    for p in blk:
        t = _f32(p)
        acc = t if acc is None else acc + t
    c = jnp.broadcast_to(-_fin(acc), acc.shape)
    sub = lax.broadcasted_iota(i32, c.shape, 0)
    return jnp.where(sub == 2, c - _hi(c), jnp.where(sub < 2, c, 0.0)).astype(bf16)


def _rows(b):
    return slice(b * RB, (b + 1) * RB)


def _prows(b):
    return slice(b * HB, (b + 1) * HB)


def _cols(s):
    return slice(s * L, (s + 1) * L)


def _dot(a, b):
    return jnp.dot(a, b, preferred_element_type=f32)


def _kernel(x_hbm, wqkv_hbm, wo_hbm, w1_hbm, w2_hbm, w3_hbm, w4t_hbm, out_hbm,
            x_v, wqkv_v, wo_v, w1_v, w2_v, w3_v, w4t_v,
            wqkvt, wot, w1t, w2t, w3t, tmp32, tmpq,
            q_s, kp, vp, h_s, h1_s, hx_s, out_v, z_a, z_b, sems):
    ng = len(_GROUPS)
    ends = {f"x{p}": (x_hbm.at[:, j0 * C:j1 * C], x_v[p].at[0:D, :]) for p, (j0, j1) in enumerate(_XP)}
    for p, nm in enumerate(("wq", "wk", "wv")):
        ends[nm] = (wqkv_hbm.at[:, _QCOLS[p][0]:_QCOLS[p][1]], wqkv_v[p])
    ends.update(wo=(wo_hbm, wo_v), w1=(w1_hbm, w1_v), w2=(w2_hbm, w2_v), w3=(w3_hbm, w3_v),
                w4=(w4t_hbm, w4t_v), z=(z_a, z_b))
    groups = [[pltpu.make_async_copy(*ends[nm], sems.at[i]) for nm in spec.split()]
              for i, spec in enumerate(_GROUPS)]
    c_out = []
    st = {}
    lane1 = lax.broadcasted_iota(i32, (8, L), 1)

    def xloc(j, s=None):
        p = [p for p, (j0, j1) in enumerate(_XP) if j0 <= j < j1][0]
        c0 = (j - _XP[p][0]) * C
        return x_v[p], (slice(c0, c0 + C) if s is None else slice(c0 + s * L, c0 + (s + 1) * L))

    def gate_bits(gate):
        return pltpu.bitcast(gate, i32) & st["zvec"]

    def gated(p, gate):
        if gate is None:
            return p
        r, c = p.shape
        gz = pltpu.bitcast(gate_bits(gate), u32)
        if c < L:
            gz = gz[:, 0:c]
        elif c > L:
            gz = jnp.concatenate([gz] * (c // L), axis=1)
        return p | jnp.broadcast_to(gz[None], (r // 8, 8, c)).reshape(r, c)

    def tied(c, res):
        t = pltpu.bitcast(pltpu.bitcast(jnp.broadcast_to(c, (8, L)), i32) | gate_bits(res), f32)
        return jnp.broadcast_to(t[None], (RB // 8, 8, L)).reshape(RB, L)

    def note(name, res):
        st.setdefault(("res", name), []).extend(
            (res, r, s) for s in range(SUB) for r in range(res.shape[0] // 8))

    def pick_gates(spec, n):
        if not spec:
            return [None] * n
        tl = []
        for item in spec.split():
            nm, _, lim = item.partition(":")
            flat = st["res", nm]
            if lim:
                lo, hi = lim.split("-")
                flat = flat[len(flat) * int(lo) // 100:len(flat) * int(hi) // 100]
            tl += flat
        out = []
        for i in range(n):
            res, r, s = tl[(i * len(tl)) // n]
            out.append(res[r * 8:(r + 1) * 8, _cols(s)])
        return out

    def windows(ref, g, b, gate, done):
        rs = slice(b * DB * 8, (b + 1) * DB * 8)
        cur, prev = ref[g + 1, rs, :], ref[g, rs, :]
        ln = lane1 | gate_bits(gate)
        if done is not None:
            ln = ln | gate_bits(done)
        for w in range(W):
            r = cur
            if w:
                mk = jnp.broadcast_to((ln < L - DIL * w)[None], (DB, 8, L)).reshape(DB * 8, L)
                r = pltpu.roll(jnp.where(mk, cur, prev), DIL * w, 1)
            t = _f32(r).reshape(DB, 2, 8, L)
            yield w, [t[:, 0], t[:, 1]]

    def att_qk(g, gates):
        lg = [[None] * W, [None] * W]
        hist = []
        for b in range(NBK):
            qb = q_s[g, b * DB * H:(b + 1) * DB * H, :].reshape(DB, 2, 8, L)
            for w, ks in windows(kp, g, b, gates[b], hist[b - 2] if b >= 2 else None):
                for i in range(2):
                    pr = jnp.sum(qb[:, i] * ks[i], axis=0)
                    lg[i][w] = pr if lg[i][w] is None else lg[i][w] + pr
            hist.append(lg[0][W - 1] + lg[1][W - 1] + lg[0][1])
        rq = st["rx", g] * (DH ** -0.5)
        a = []
        for i in range(2):
            sc = [t * rq for t in lg[i]]
            if g == 0:
                sc = [jnp.where(lane1 >= DIL * w, sc[w], -1e9) for w in range(W)]
            m = functools.reduce(jnp.maximum, sc)
            p = [jnp.exp(s_ - m) for s_ in sc]
            r = 1.0 / functools.reduce(jnp.add, p)
            a.append([p_ * r for p_ in p])
        st["att", g] = a

    def att_pv(g, gates):
        a = st["att", g]
        ob = []
        for b in range(NBK):
            o = [None, None]
            done = ob[b - 2][0:8] + ob[b - 2][DB * H - 8:] if b >= 2 else None
            for w, vs in windows(vp, g, b, gates[b], done):
                for i in range(2):
                    t = a[i][w][None] * vs[i]
                    o[i] = t if o[i] is None else o[i] + t
            ob.append(jnp.stack(o, axis=1).reshape(DB * H, L))
        st["o", g] = jnp.concatenate(ob, axis=0)

    def t_a(j, spec):
        gates = pick_gates(spec, SUB * 2 * NBK)
        for s in range(SUB):
            att_qk(j * SUB + s, gates[2 * s * NBK:(2 * s + 1) * NBK])
            att_pv(j * SUB + s, gates[(2 * s + 1) * NBK:(2 * s + 2) * NBK])

    def t_c(g, spec):
        att_qk(g, pick_gates(spec, NBK))

    def t_d(g, spec):
        att_pv(g, pick_gates(spec, NBK))

    def cat(key, j, rs=slice(None)):
        return jnp.concatenate([st[key, j * SUB + s][rs] for s in range(SUB)], axis=1).astype(bf16)

    def t_l(j, spec=None):
        gates = pick_gates(spec, SUB * NB)
        for s in range(SUB):
            xr, cs = xloc(j, s)
            a1 = a2 = None
            for b in range(NB):
                x = _f32(gated(_pk(xr[_rows(b), cs]), gates[s * NB + b]))
                a1 = x if a1 is None else a1 + x
                a2 = x * x if a2 is None else a2 + x * x
            m, v = _stats(a1, a2)
            st["rx", j * SUB + s] = lax.rsqrt(v + EPS)
            xr[D:DA, cs] = _mean_rows(m).astype(bf16)

    def qkv_epi(j, part, res):
        for s in range(SUB):
            g = j * SUB + s
            if part == 0:
                q_s[g] = res[:, _cols(s)]
            else:
                dst = kp if part == 1 else vp
                dst[g + 1] = _pk((res[:, _cols(s)] * st["rx", g]).astype(bf16))

    def t_Q(j):
        xr, cs = xloc(j)
        qkv = _dot(_up(wqkvt[...]), xr[:, cs])
        note(f"Q{j}", qkv)
        for p in range(3):
            qkv_epi(j, p, qkv[p * D:(p + 1) * D])

    def t_part(p, j):
        xr, cs = xloc(j)
        res = _dot(_up(wqkvt[p * D // 2:(p + 1) * D // 2, :]), xr[:, cs])
        note("qkv"[p] + str(j), res)
        qkv_epi(j, p, res)

    def t_O(j):
        ao = _dot(_up(wot[...]), cat("o", j))
        note(f"O{j}", ao)
        for s in range(SUB):
            g = j * SUB + s
            xr, cs = xloc(j, s)
            a1 = a2 = None
            hb = []
            done = None
            for b in range(NB):
                h = _f32(gated(_pk(xr[_rows(b), cs]), done)) + ao[_rows(b), _cols(s)]
                h_s[g, _rows(b), :] = h
                hb.append(h)
                a1 = h if a1 is None else a1 + h
                a2 = h * h if a2 is None else a2 + h * h
                done = jnp.sum((a1 + a2).reshape(RB // 8, 8, L), axis=0)
            m, v = _stats(a1, a2)
            r = lax.rsqrt(v + EPS)
            r2 = lax.rsqrt(v * r * r + EPS)
            st["h", g] = (m, r, _gelu_coef(r * r2))
            st["hb", g] = jnp.concatenate(hb + [_mean_rows(m)], axis=0)

    def t_M(j):
        a1 = _dot(_up(w1t[...]), cat("hb", j))
        note(f"M{j}", a1)
        for s in range(SUB):
            g = j * SUB + s
            ca, cb, ch = st["h", g][2]
            h1 = []
            for b in range(NB):
                y = a1[_rows(b), _cols(s)]
                hy = y * ch
                h1.append(hy + hy * jnp.tanh(y * (ca + cb * (y * y))))
            h1_s[g + 1] = _pk(jnp.concatenate(h1, axis=0).astype(bf16))

    grp = D // 8
    lane_g = lax.broadcasted_iota(i32, (grp, L), 1)

    def t_s(j):
        for s in range(SUB):
            g = j * SUB + s + 1
            parts = []
            for gi, sh in enumerate((1, -1, 2, -2)):
                gs = slice(gi * grp, (gi + 1) * grp)
                if sh > 0:
                    r = pltpu.roll(jnp.where(lane_g < L - sh, h1_s[g, gs, :], h1_s[g - 1, gs, :]), sh, 1)
                else:
                    r = pltpu.roll(jnp.where(lane_g >= -sh, h1_s[g, gs, :], h1_s[g + 1, gs, :]), L + sh, 1)
                parts.append(r)
            st["hsh", g - 1] = _up(jnp.concatenate(parts, axis=0))

    def t_P(j):
        hs = _dot(_up(w2t[...]), cat("hsh", j))
        note(f"P{j}", hs)
        for s in range(SUB):
            g = j * SUB + s
            m, r, _ = st["h", g]
            a1 = a2 = None
            xb = []
            for b in range(NB):
                h = h_s[g, _rows(b), :]
                x1 = (h - (tied(m, done) if b else m)) * r + hs[_rows(b), _cols(s)]
                hx_s[g, _rows(b), :] = h + x1
                xb.append(x1)
                a1 = x1 if a1 is None else a1 + x1
                a2 = x1 * x1 if a2 is None else a2 + x1 * x1
                done = jnp.sum((a1 + a2).reshape(RB // 8, 8, L), axis=0)
            m3, v3 = _stats(a1, a2)
            st["x", g] = _gelu_coef(lax.rsqrt(v3 + EPS))
            st["xb", g] = jnp.concatenate(xb + [_mean_rows(m3)], axis=0)

    def t_U(j):
        a3 = _dot(_up(w3t[...]), cat("xb", j))
        note(f"U{j}", a3)
        for s in range(SUB):
            ca, cb, _ = st["x", j * SUB + s]
            gb = []
            for b in range(F // RB):
                y = a3[_rows(b), _cols(s)]
                gb.append(y * (1.0 + jnp.tanh(y * (ca + cb * (y * y)))))
            st["g", j * SUB + s] = jnp.concatenate(gb, axis=0)

    def t_V(j):
        halves = ((0, NB // 2), (NB // 2, NB)) if j == NC - 1 else ((0, NB),)
        gj = {c: cat("g", j, slice(c, min(c + 512, F))) for c in range(0, F, 512)}
        for hi, (b0, b1) in enumerate(halves):
            h2 = None
            for c in range(0, F, 512):
                e = min(c + 512, F)
                t = _dot(w4t_v[b0 * RB:b1 * RB, c:e], gj[c])
                note(f"V{j}", t)
                h2 = t if h2 is None else h2 + t
            for s in range(SUB):
                g = j * SUB + s
                ov = out_v[g + hi * SUB]
                ch = st["x", g][2]
                ov[...] = (hx_s[g, b0 * RB:b1 * RB, :] + h2[:, _cols(s)] * ch).astype(bf16)
                cp = pltpu.make_async_copy(ov, out_hbm.at[b0 * RB:b1 * RB, _cols(g)], sems.at[ng])
                cp.start()
                c_out.append(cp)

    def t_W(i):
        if i == 0:
            z_a[...] = jnp.zeros((8, L), i32)
            for group in groups:
                for c in group:
                    c.start()
            kp[0] = jnp.zeros((D // 2, L), u32)
            vp[0] = jnp.zeros((D // 2, L), u32)
            h1_s[0] = jnp.zeros((D // 2, L), u32)
            h1_s[NT + 1] = jnp.zeros((D // 2, L), u32)
        for c in groups[i]:
            c.wait()
        if i == 1:
            st["zvec"] = z_b[...]

    def t_Xpart(p):
        c0, c1 = _QCOLS[p]
        blk = [_pk(wqkv_v[p][b * 16:(b + 1) * 16, :]) for b in range(D // 16)]
        src = jnp.concatenate([_up(p_) for p_ in blk] + [_colsum_rows(blk)], axis=0).T.astype(f32)
        for c4 in range(4):
            wd = min(L, DA - c4 * L)
            tmpq[c4, c0:c1, 0:wd] = src[:, c4 * L:c4 * L + wd]
        for d in range(DH):
            for c4 in range(4):
                wd = min(L, DA - c4 * L)
                wqkvt[(p * D + d * H) // 2:(p * D + (d + 1) * H) // 2, c4 * L:c4 * L + wd] = (
                    _pk(tmpq[c4, pl.ds(p * D + d, H, stride=DH), 0:wd].astype(bf16)))

    def t_Xo(spec):
        gates = pick_gates(spec, 8)
        for c4 in range(4):
            wd = min(L, D - c4 * L)
            cs = slice(c4 * L, c4 * L + wd)
            for hf in range(2):
                p = gated(_pk(wo_v[hf * 224:(hf + 1) * 224, cs]), gates[c4 * 2 + hf])
                tmp32[c4, hf * 224:(hf + 1) * 224, 0:wd] = _f32(p)
            t = jnp.concatenate([tmp32[c4, pl.ds(d, H, stride=DH), 0:wd].astype(bf16) for d in range(DH)], axis=0)
            wot[c4 * L // 2:(c4 * L + wd) // 2, :] = _pk(t.T)

    def xpose_w(w_v, dst, n, xw, aug, spec):
        nb = -(-n // xw)
        gates = pick_gates(spec, nb * 4)
        for c in range(nb):
            c0, c1 = c * xw, min((c + 1) * xw, n)
            blk = [gated(_pk(w_v[b * 16:(b + 1) * 16, c0:c1]), gates[c * 4 + b // 7]) for b in range(D // 16)]
            t = jnp.concatenate([_up(p_) for p_ in blk] + ([_colsum_rows(blk)] if aug else []), axis=0)
            dst[c0 // 2:c1 // 2, :] = _pk(t.T)

    part = functools.partial
    once = dict(Xq=part(t_Xpart, 0), Xk=part(t_Xpart, 1), Xv=part(t_Xpart, 2), Xo=t_Xo,
                X1=part(xpose_w, w1_v, w1t, D, L, True), X2=part(xpose_w, w2_v, w2t, D, L, False),
                X3=part(xpose_w, w3_v, w3t, F, 256, True))
    per = dict(a=t_a, c=t_c, d=t_d, l=t_l, Q=t_Q, O=t_O, M=t_M, s=t_s, P=t_P, U=t_U, V=t_V, W=t_W,
               q=part(t_part, 0), k=part(t_part, 1), v=part(t_part, 2))
    for task in _ORDER:
        name, extra = (task[0], task[1:]) if isinstance(task, tuple) else (task, ())
        if name in once:
            once[name](*extra)
        else:
            per[name[0]](int(name[1:]), *extra)
    for c in c_out:
        c.wait()


@jax.jit
def pallas_sequential_preLN__sliding_local_dilated__mixer_s_mlp__prompt_kernel(
    A_x: jax.Array,
    A_wqkv: jax.Array,
    A_wo: jax.Array,
    B_x: jax.Array,
    B_w1: jax.Array,
    B_w2: jax.Array,
    B_w3: jax.Array,
    B_w4: jax.Array,
):
    del B_x
    hbm = pl.BlockSpec(memory_space=pl.ANY)
    V = pltpu.VMEM
    out_t = pl.pallas_call(
        _kernel,
        in_specs=[hbm] * 7,
        out_specs=hbm,
        out_shape=jax.ShapeDtypeStruct((D, S), bf16),
        scratch_shapes=[
            [V((DA, (j1 - j0) * C), bf16) for j0, j1 in _XP],
            [V((D, c1 - c0), bf16) for c0, c1 in _QCOLS],
            V((D, D), bf16), V((D, D), bf16),
            V((D, D), bf16), V((D, F), bf16), V((D, F), bf16),
            V((3 * D // 2, DA), u32), V((D // 2, D), u32), V((D // 2, DA), u32),
            V((D // 2, D), u32), V((F // 2, DA), u32),
            V((4, D, L), f32), V((4, 3 * D, L), f32),
            V((NT, D, L), f32), V((NT + 1, D // 2, L), u32), V((NT + 1, D // 2, L), u32),
            V((NT, D, L), f32), V((NT + 2, D // 2, L), u32), V((NT, D, L), f32),
            [V((D, L), bf16)] * (NT - SUB) + [V((D // 2, L), bf16)] * (2 * SUB),
            V((8, L), i32), V((8, L), i32),
            pltpu.SemaphoreType.DMA((len(_GROUPS) + 1,)),
        ],
        compiler_params=pltpu.CompilerParams(
            vmem_limit_bytes=100 * 1024 * 1024, disable_semaphore_checks=True),
    )(A_x.reshape(S, D).T, A_wqkv, A_wo, B_w1, B_w2, B_w3, B_w4.T)
    return out_t.T.reshape(1, S, D)
```

```python
import functools

import jax
import jax.numpy as jnp
from jax import lax
from jax.experimental import pallas as pl
from jax.experimental.pallas import tpu as pltpu

S, D, F, H, DH, W, DIL = 2048, 448, 1792, 16, 28, 8, 2
DA = D + 16
EPS = 1e-5
f32, bf16, u32, i32 = jnp.float32, jnp.bfloat16, jnp.uint32, jnp.int32
L = 128
NT = S // L
C = 256
NC = S // C
SUB = C // L
RB = 32
HB = RB // 2
NB = D // RB
DB = 4
NBK = DH // DB
_C0 = 0.7978845608028654
_C1 = 0.044715
_QCOLS = ((0, 512), (512, 896), (896, 3 * D))
_XP = ((0, 1), (1, 3), (3, 4), (4, 5), (5, 8))
_LAST = ((0, 10), (10, NB))

_GROUPS = ("wq", "x0 z", "x1", "wk x2", "wv wo w1 w2 x3", "w3 w4 x4")


def _order():
    o = ["W0", "Xq", "W1", "l0", "q0",
         "W2", "l1", "q1", ("l2", "q1:0-60"), "q2",
         "W3", "l3", "q3", "Xk", "k0", "k1", "k2", "k3",
         ("c0", "k0:60-100 k1:0-60"), ("c1", "k1:60-100 k2:0-60"), ("c2", "k2:60-100 k3:0-60"),
         "W4", "l4", "q4", "Xv", "k4", "v0", "v1", "v2", "v3", "v4",
         ("c3", "k4"), ("Xo", "v0 v1"), ("X1", "v2 v3"),
         ("d0", "v1"), ("d1", "v2"), ("d2", "v3"), ("d3", "v4"),
         "O0", "M0", "O1", "M1", ("X2", "O0 M0 O1"), "s0",
         "W5", "P0", ("l5", "P0:0-60"), "Q5", ("X3", "P0 Q5:0-80"), "U0", "V0",
         ("a2", "U0 V0:0-70")]
    for n in range(2, NC - 1):
        q = n + 4 < NC
        o += [f"O{n}"] + ([(f"l{n+4}", f"O{n}")] if q else []) + [f"M{n}", f"s{n-1}"]
        o += ([f"Q{n+4}"] if q else []) + [f"P{n-1}", f"U{n-1}", f"V{n-1}"]
        o += [(f"a{n+1}", (f"Q{n+4} " if q else "") + f"U{n-1} V{n-1}:0-70")]
    n = NC - 1
    o += [f"O{n}", f"M{n}", f"s{n-1}", f"P{n-1}", f"s{n}", f"P{n}", f"U{n-1}", f"V{n-1}", f"U{n}", f"V{n}"]
    return o


_ORDER = _order()


def _gelu_coef(sc):
    return _C0 * sc, (_C0 * _C1) * (sc * sc * sc), 0.5 * sc


def _pk(x):
    return pltpu.bitcast(x, u32)


def _up(x):
    return pltpu.bitcast(x, bf16)


def _f32(p):
    return _up(p).astype(f32)


def _hi(x):
    return x.astype(bf16).astype(f32)


def _fin(acc):
    return jnp.sum(acc, axis=0, keepdims=True)


def _stats(a1, a2):
    m = _fin(a1) * (1.0 / D)
    v = jnp.maximum(_fin(a2) * (1.0 / D) - m * m, 0.0)
    return m, v


def _mean_rows(m):
    mb = jnp.broadcast_to(m, (16, m.shape[1]))
    sub = lax.broadcasted_iota(i32, mb.shape, 0)
    return jnp.where(sub == 1, mb - _hi(mb), jnp.where(sub < 3, mb, 0.0))


def _colsum_rows(blk):
    acc = None
    for p in blk:
        t = _f32(p)
        acc = t if acc is None else acc + t
    c = jnp.broadcast_to(-_fin(acc), acc.shape)
    sub = lax.broadcasted_iota(i32, c.shape, 0)
    return jnp.where(sub == 2, c - _hi(c), jnp.where(sub < 2, c, 0.0)).astype(bf16)


def _rows(b):
    return slice(b * RB, (b + 1) * RB)


def _prows(b):
    return slice(b * HB, (b + 1) * HB)


def _cols(s):
    return slice(s * L, (s + 1) * L)


def _dot(a, b):
    return jnp.dot(a, b, preferred_element_type=f32)


def _kernel(x_hbm, wqkv_hbm, wo_hbm, w1_hbm, w2_hbm, w3_hbm, w4t_hbm, out_hbm,
            x_v, wqkv_v, wo_v, w1_v, w2_v, w3_v, w4t_v,
            wqkvt, wot, w1t, w2t, w3t, tmp32, tmpq,
            q_s, kp, vp, h_s, h1_s, hx_s, out_v, z_a, z_b, sems):
    ng = len(_GROUPS)
    ends = {f"x{p}": (x_hbm.at[:, j0 * C:j1 * C], x_v[p].at[0:D, :]) for p, (j0, j1) in enumerate(_XP)}
    for p, nm in enumerate(("wq", "wk", "wv")):
        ends[nm] = (wqkv_hbm.at[:, _QCOLS[p][0]:_QCOLS[p][1]], wqkv_v[p])
    ends.update(wo=(wo_hbm, wo_v), w1=(w1_hbm, w1_v), w2=(w2_hbm, w2_v), w3=(w3_hbm, w3_v),
                w4=(w4t_hbm, w4t_v), z=(z_a, z_b))
    groups = [[pltpu.make_async_copy(*ends[nm], sems.at[i]) for nm in spec.split()]
              for i, spec in enumerate(_GROUPS)]
    c_out = []
    st = {}
    lane1 = lax.broadcasted_iota(i32, (8, L), 1)

    def xloc(j, s=None):
        p = [p for p, (j0, j1) in enumerate(_XP) if j0 <= j < j1][0]
        c0 = (j - _XP[p][0]) * C
        return x_v[p], (slice(c0, c0 + C) if s is None else slice(c0 + s * L, c0 + (s + 1) * L))

    def gate_bits(gate):
        return pltpu.bitcast(gate, i32) & st["zvec"]

    def gated(p, gate):
        if gate is None:
            return p
        r, c = p.shape
        gz = pltpu.bitcast(gate_bits(gate), u32)
        if c < L:
            gz = gz[:, 0:c]
        elif c > L:
            gz = jnp.concatenate([gz] * (c // L), axis=1)
        return p | jnp.broadcast_to(gz[None], (r // 8, 8, c)).reshape(r, c)

    def tied(c, res):
        t = pltpu.bitcast(pltpu.bitcast(jnp.broadcast_to(c, (8, L)), i32) | gate_bits(res), f32)
        return jnp.broadcast_to(t[None], (RB // 8, 8, L)).reshape(RB, L)

    def note(name, res):
        st.setdefault(("res", name), []).extend(
            (res, r, s) for s in range(SUB) for r in range(res.shape[0] // 8))

    def pick_gates(spec, n):
        if not spec:
            return [None] * n
        tl = []
        for item in spec.split():
            nm, _, lim = item.partition(":")
            flat = st["res", nm]
            if lim:
                lo, hi = lim.split("-")
                flat = flat[len(flat) * int(lo) // 100:len(flat) * int(hi) // 100]
            tl += flat
        out = []
        for i in range(n):
            res, r, s = tl[(i * len(tl)) // n]
            out.append(res[r * 8:(r + 1) * 8, _cols(s)])
        return out

    def windows(ref, g, b, gate, done):
        rs = slice(b * DB * 8, (b + 1) * DB * 8)
        cur, prev = ref[g + 1, rs, :], ref[g, rs, :]
        ln = lane1 | gate_bits(gate)
        if done is not None:
            ln = ln | gate_bits(done)
        for w in range(W):
            r = cur
            if w:
                mk = jnp.broadcast_to((ln < L - DIL * w)[None], (DB, 8, L)).reshape(DB * 8, L)
                r = pltpu.roll(jnp.where(mk, cur, prev), DIL * w, 1)
            t = _f32(r).reshape(DB, 2, 8, L)
            yield w, [t[:, 0], t[:, 1]]

    def att_qk(g, gates):
        lg = [[None] * W, [None] * W]
        hist = []
        for b in range(NBK):
            qb = q_s[g, b * DB * H:(b + 1) * DB * H, :].reshape(DB, 2, 8, L)
            for w, ks in windows(kp, g, b, gates[b], hist[b - 2] if b >= 2 else None):
                for i in range(2):
                    pr = jnp.sum(qb[:, i] * ks[i], axis=0)
                    lg[i][w] = pr if lg[i][w] is None else lg[i][w] + pr
            hist.append(lg[0][W - 1] + lg[1][W - 1] + lg[0][1])
        rq = st["rx", g] * (DH ** -0.5)
        a = []
        for i in range(2):
            sc = [t * rq for t in lg[i]]
            if g == 0:
                sc = [jnp.where(lane1 >= DIL * w, sc[w], -1e9) for w in range(W)]
            m = functools.reduce(jnp.maximum, sc)
            p = [jnp.exp(s_ - m) for s_ in sc]
            r = 1.0 / functools.reduce(jnp.add, p)
            a.append([p_ * r for p_ in p])
        st["att", g] = a

    def att_pv(g, gates):
        a = st["att", g]
        ob = []
        for b in range(NBK):
            o = [None, None]
            done = ob[b - 2][0:8] + ob[b - 2][DB * H - 8:] if b >= 2 else None
            for w, vs in windows(vp, g, b, gates[b], done):
                for i in range(2):
                    t = a[i][w][None] * vs[i]
                    o[i] = t if o[i] is None else o[i] + t
            ob.append(jnp.stack(o, axis=1).reshape(DB * H, L))
        st["o", g] = jnp.concatenate(ob, axis=0)

    def t_a(j, spec):
        gates = pick_gates(spec, SUB * 2 * NBK)
        for s in range(SUB):
            att_qk(j * SUB + s, gates[2 * s * NBK:(2 * s + 1) * NBK])
            att_pv(j * SUB + s, gates[(2 * s + 1) * NBK:(2 * s + 2) * NBK])

    def t_c(g, spec):
        att_qk(g, pick_gates(spec, NBK))

    def t_d(g, spec):
        att_pv(g, pick_gates(spec, NBK))

    def cat(key, j, rs=slice(None)):
        return jnp.concatenate([st[key, j * SUB + s][rs] for s in range(SUB)], axis=1).astype(bf16)

    def t_l(j, spec=None):
        gates = pick_gates(spec, SUB * NB)
        for s in range(SUB):
            xr, cs = xloc(j, s)
            a1 = a2 = None
            for b in range(NB):
                x = _f32(gated(_pk(xr[_rows(b), cs]), gates[s * NB + b]))
                a1 = x if a1 is None else a1 + x
                a2 = x * x if a2 is None else a2 + x * x
            m, v = _stats(a1, a2)
            st["rx", j * SUB + s] = lax.rsqrt(v + EPS)
            xr[D:DA, cs] = _mean_rows(m).astype(bf16)

    def qkv_epi(j, part, res):
        for s in range(SUB):
            g = j * SUB + s
            if part == 0:
                q_s[g] = res[:, _cols(s)]
            else:
                dst = kp if part == 1 else vp
                dst[g + 1] = _pk((res[:, _cols(s)] * st["rx", g]).astype(bf16))

    def t_Q(j):
        xr, cs = xloc(j)
        qkv = _dot(_up(wqkvt[...]), xr[:, cs])
        note(f"Q{j}", qkv)
        for p in range(3):
            qkv_epi(j, p, qkv[p * D:(p + 1) * D])

    def t_part(p, j):
        xr, cs = xloc(j)
        res = _dot(_up(wqkvt[p * D // 2:(p + 1) * D // 2, :]), xr[:, cs])
        note("qkv"[p] + str(j), res)
        qkv_epi(j, p, res)

    def t_O(j):
        ao = _dot(_up(wot[...]), cat("o", j))
        note(f"O{j}", ao)
        for s in range(SUB):
            g = j * SUB + s
            xr, cs = xloc(j, s)
            a1 = a2 = None
            hb = []
            done = None
            for b in range(NB):
                h = _f32(gated(_pk(xr[_rows(b), cs]), done)) + ao[_rows(b), _cols(s)]
                h_s[g, _rows(b), :] = h
                hb.append(h)
                a1 = h if a1 is None else a1 + h
                a2 = h * h if a2 is None else a2 + h * h
                done = jnp.sum((a1 + a2).reshape(RB // 8, 8, L), axis=0)
            m, v = _stats(a1, a2)
            r = lax.rsqrt(v + EPS)
            r2 = lax.rsqrt(v * r * r + EPS)
            st["h", g] = (m, r, _gelu_coef(r * r2))
            st["hb", g] = jnp.concatenate(hb + [_mean_rows(m)], axis=0)

    def t_M(j):
        a1 = _dot(_up(w1t[...]), cat("hb", j))
        note(f"M{j}", a1)
        for s in range(SUB):
            g = j * SUB + s
            ca, cb, ch = st["h", g][2]
            h1 = []
            for b in range(NB):
                y = a1[_rows(b), _cols(s)]
                hy = y * ch
                h1.append(hy + hy * jnp.tanh(y * (ca + cb * (y * y))))
            h1_s[g + 1] = _pk(jnp.concatenate(h1, axis=0).astype(bf16))

    grp = D // 8
    lane_g = lax.broadcasted_iota(i32, (grp, L), 1)

    def t_s(j):
        for s in range(SUB):
            g = j * SUB + s + 1
            parts = []
            for gi, sh in enumerate((1, -1, 2, -2)):
                gs = slice(gi * grp, (gi + 1) * grp)
                if sh > 0:
                    r = pltpu.roll(jnp.where(lane_g < L - sh, h1_s[g, gs, :], h1_s[g - 1, gs, :]), sh, 1)
                else:
                    r = pltpu.roll(jnp.where(lane_g >= -sh, h1_s[g, gs, :], h1_s[g + 1, gs, :]), L + sh, 1)
                parts.append(r)
            st["hsh", g - 1] = _up(jnp.concatenate(parts, axis=0))

    def t_P(j):
        hs = _dot(_up(w2t[...]), cat("hsh", j))
        note(f"P{j}", hs)
        for s in range(SUB):
            g = j * SUB + s
            m, r, _ = st["h", g]
            a1 = a2 = None
            xb = []
            for b in range(NB):
                h = h_s[g, _rows(b), :]
                x1 = (h - (tied(m, done) if b else m)) * r + hs[_rows(b), _cols(s)]
                hx_s[g, _rows(b), :] = h + x1
                xb.append(x1)
                a1 = x1 if a1 is None else a1 + x1
                a2 = x1 * x1 if a2 is None else a2 + x1 * x1
                done = jnp.sum((a1 + a2).reshape(RB // 8, 8, L), axis=0)
            m3, v3 = _stats(a1, a2)
            st["x", g] = _gelu_coef(lax.rsqrt(v3 + EPS))
            st["xb", g] = jnp.concatenate(xb + [_mean_rows(m3)], axis=0)

    def t_U(j):
        a3 = _dot(_up(w3t[...]), cat("xb", j))
        note(f"U{j}", a3)
        for s in range(SUB):
            ca, cb, _ = st["x", j * SUB + s]
            gb = []
            for b in range(F // RB):
                y = a3[_rows(b), _cols(s)]
                gb.append(y * (1.0 + jnp.tanh(y * (ca + cb * (y * y)))))
            st["g", j * SUB + s] = jnp.concatenate(gb, axis=0)

    def t_V(j):
        pieces = _LAST if j == NC - 1 else ((0, NB),)
        gj = {c: cat("g", j, slice(c, min(c + 512, F))) for c in range(0, F, 512)}
        for pi, (b0, b1) in enumerate(pieces):
            h2 = None
            for c in range(0, F, 512):
                e = min(c + 512, F)
                t = _dot(w4t_v[b0 * RB:b1 * RB, c:e], gj[c])
                note(f"V{j}", t)
                h2 = t if h2 is None else h2 + t
            for s in range(SUB):
                g = j * SUB + s
                ov = out_v[g + pi * SUB]
                ch = st["x", g][2]
                ov[...] = (hx_s[g, b0 * RB:b1 * RB, :] + h2[:, _cols(s)] * ch).astype(bf16)
                cp = pltpu.make_async_copy(ov, out_hbm.at[b0 * RB:b1 * RB, _cols(g)], sems.at[ng])
                cp.start()
                c_out.append(cp)

    def t_W(i):
        if i == 0:
            z_a[...] = jnp.zeros((8, L), i32)
            for group in groups:
                for c in group:
                    c.start()
            kp[0] = jnp.zeros((D // 2, L), u32)
            vp[0] = jnp.zeros((D // 2, L), u32)
            h1_s[0] = jnp.zeros((D // 2, L), u32)
            h1_s[NT + 1] = jnp.zeros((D // 2, L), u32)
        for c in groups[i]:
            c.wait()
        if i == 1:
            st["zvec"] = z_b[...]

    def t_Xpart(p):
        c0, c1 = _QCOLS[p]
        blk = [_pk(wqkv_v[p][b * 16:(b + 1) * 16, :]) for b in range(D // 16)]
        src = jnp.concatenate([_up(p_) for p_ in blk] + [_colsum_rows(blk)], axis=0).T.astype(f32)
        for c4 in range(4):
            wd = min(L, DA - c4 * L)
            tmpq[c4, c0:c1, 0:wd] = src[:, c4 * L:c4 * L + wd]
        for d in range(DH):
            for c4 in range(4):
                wd = min(L, DA - c4 * L)
                wqkvt[(p * D + d * H) // 2:(p * D + (d + 1) * H) // 2, c4 * L:c4 * L + wd] = (
                    _pk(tmpq[c4, pl.ds(p * D + d, H, stride=DH), 0:wd].astype(bf16)))

    def t_Xo(spec):
        gates = pick_gates(spec, 8)
        for c4 in range(4):
            wd = min(L, D - c4 * L)
            cs = slice(c4 * L, c4 * L + wd)
            for hf in range(2):
                p = gated(_pk(wo_v[hf * 224:(hf + 1) * 224, cs]), gates[c4 * 2 + hf])
                tmp32[c4, hf * 224:(hf + 1) * 224, 0:wd] = _f32(p)
            t = jnp.concatenate([tmp32[c4, pl.ds(d, H, stride=DH), 0:wd].astype(bf16) for d in range(DH)], axis=0)
            wot[c4 * L // 2:(c4 * L + wd) // 2, :] = _pk(t.T)

    def xpose_w(w_v, dst, n, xw, aug, spec):
        nb = -(-n // xw)
        gates = pick_gates(spec, nb * 4)
        for c in range(nb):
            c0, c1 = c * xw, min((c + 1) * xw, n)
            blk = [gated(_pk(w_v[b * 16:(b + 1) * 16, c0:c1]), gates[c * 4 + b // 7]) for b in range(D // 16)]
            t = jnp.concatenate([_up(p_) for p_ in blk] + ([_colsum_rows(blk)] if aug else []), axis=0)
            dst[c0 // 2:c1 // 2, :] = _pk(t.T)

    part = functools.partial
    once = dict(Xq=part(t_Xpart, 0), Xk=part(t_Xpart, 1), Xv=part(t_Xpart, 2), Xo=t_Xo,
                X1=part(xpose_w, w1_v, w1t, D, L, True), X2=part(xpose_w, w2_v, w2t, D, L, False),
                X3=part(xpose_w, w3_v, w3t, F, 256, True))
    per = dict(a=t_a, c=t_c, d=t_d, l=t_l, Q=t_Q, O=t_O, M=t_M, s=t_s, P=t_P, U=t_U, V=t_V, W=t_W,
               q=part(t_part, 0), k=part(t_part, 1), v=part(t_part, 2))
    for task in _ORDER:
        name, extra = (task[0], task[1:]) if isinstance(task, tuple) else (task, ())
        if name in once:
            once[name](*extra)
        else:
            per[name[0]](int(name[1:]), *extra)
    for c in c_out:
        c.wait()


@jax.jit
def pallas_sequential_preLN__sliding_local_dilated__mixer_s_mlp__prompt_kernel(
    A_x: jax.Array,
    A_wqkv: jax.Array,
    A_wo: jax.Array,
    B_x: jax.Array,
    B_w1: jax.Array,
    B_w2: jax.Array,
    B_w3: jax.Array,
    B_w4: jax.Array,
):
    del B_x
    hbm = pl.BlockSpec(memory_space=pl.ANY)
    V = pltpu.VMEM
    out_t = pl.pallas_call(
        _kernel,
        in_specs=[hbm] * 7,
        out_specs=hbm,
        out_shape=jax.ShapeDtypeStruct((D, S), bf16),
        scratch_shapes=[
            [V((DA, (j1 - j0) * C), bf16) for j0, j1 in _XP],
            [V((D, c1 - c0), bf16) for c0, c1 in _QCOLS],
            V((D, D), bf16), V((D, D), bf16),
            V((D, D), bf16), V((D, F), bf16), V((D, F), bf16),
            V((3 * D // 2, DA), u32), V((D // 2, D), u32), V((D // 2, DA), u32),
            V((D // 2, D), u32), V((F // 2, DA), u32),
            V((4, D, L), f32), V((4, 3 * D, L), f32),
            V((NT, D, L), f32), V((NT + 1, D // 2, L), u32), V((NT + 1, D // 2, L), u32),
            V((NT, D, L), f32), V((NT + 2, D // 2, L), u32), V((NT, D, L), f32),
            [V((D, L), bf16)] * (NT - SUB)
            + [V(((b1 - b0) * RB, L), bf16) for b0, b1 in _LAST for _ in range(SUB)],
            V((8, L), i32), V((8, L), i32),
            pltpu.SemaphoreType.DMA((len(_GROUPS) + 1,)),
        ],
        compiler_params=pltpu.CompilerParams(
            vmem_limit_bytes=100 * 1024 * 1024, disable_semaphore_checks=True),
    )(A_x.reshape(S, D).T, A_wqkv, A_wo, B_w1, B_w2, B_w3, B_w4.T)
    return out_t.T.reshape(1, S, D)
```

```python
import functools

import jax
import jax.numpy as jnp
from jax import lax
from jax.experimental import pallas as pl
from jax.experimental.pallas import tpu as pltpu

S, D, F, H, DH, W, DIL = 2048, 448, 1792, 16, 28, 8, 2
DA = D + 16
EPS = 1e-5
f32, bf16, u32, i32 = jnp.float32, jnp.bfloat16, jnp.uint32, jnp.int32
L = 128
NT = S // L
C = 256
NC = S // C
SUB = C // L
RB = 32
NB = D // RB
DB = 4
NBK = DH // DB
_C0 = 0.7978845608028654
_C1 = 0.044715
_QCOLS = ((0, 512), (512, 896), (896, 3 * D))
_XP = ((0, 1), (1, 3), (3, 4), (4, 5), (5, 8))
_LAST = ((0, 10), (10, NB))

_GROUPS = ("wq", "x0 z", "x1", "wk x2", "wv wo w1 w2 x3", "w3 w4 x4")


def _order():
    o = ["W0", "Xq", "W1", "l0", "q0",
         "W2", "l1", "q1", ("l2", "q1:0-60"), "q2",
         "W3", "l3", "q3", "Xk", "k0", "k1", "k2", "k3",
         ("c0", "k0:60-100 k1:0-60"), ("c1", "k1:60-100 k2:0-60"), ("c2", "k2:60-100 k3:0-60"),
         "W4", "l4", "q4", "Xv", "k4", "v0", "v1", "v2", "v3", "v4",
         ("c3", "k4"), ("Xo", "v0 v1"), ("X1", "v2 v3"),
         ("d0", "v1"), ("d1", "v2"), ("d2", "v3"), ("d3", "v4"),
         "O0", "M0", "O1", "M1", ("X2", "O0 M0 O1"), "s0",
         "W5", "P0", ("l5", "P0:0-60"), "Q5", ("X3", "P0 Q5:0-80"), "U0", "V0",
         ("a2", "U0 V0:0-70")]
    for n in range(2, NC - 1):
        q = n + 4 < NC
        o += [f"O{n}"] + ([(f"l{n+4}", f"O{n}")] if q else []) + [f"M{n}", f"s{n-1}"]
        o += ([f"Q{n+4}"] if q else []) + [f"P{n-1}", f"U{n-1}", f"V{n-1}"]
        o += [(f"a{n+1}", (f"Q{n+4} " if q else "") + f"U{n-1} V{n-1}:0-70")]
    n = NC - 1
    o += [f"O{n}", f"M{n}", f"s{n-1}", f"P{n-1}", f"s{n}", f"P{n}", f"U{n-1}", f"V{n-1}", f"U{n}", f"V{n}"]
    return o


_ORDER = _order()


def _gelu_coef(sc):
    return _C0 * sc, (_C0 * _C1) * (sc * sc * sc), 0.5 * sc


def _pk(x):
    return pltpu.bitcast(x, u32)


def _up(x):
    return pltpu.bitcast(x, bf16)


def _f32(p):
    return _up(p).astype(f32)


def _hi(x):
    return x.astype(bf16).astype(f32)


def _fin(acc):
    return jnp.sum(acc, axis=0, keepdims=True)


def _stats(a1, a2):
    m = _fin(a1) * (1.0 / D)
    v = jnp.maximum(_fin(a2) * (1.0 / D) - m * m, 0.0)
    return m, v


def _mean_rows(m):
    mb = jnp.broadcast_to(m, (16, m.shape[1]))
    sub = lax.broadcasted_iota(i32, mb.shape, 0)
    return jnp.where(sub == 1, mb - _hi(mb), jnp.where(sub < 3, mb, 0.0))


def _colsum_rows(blk):
    acc = None
    for p in blk:
        t = _f32(p)
        acc = t if acc is None else acc + t
    c = jnp.broadcast_to(-_fin(acc), acc.shape)
    sub = lax.broadcasted_iota(i32, c.shape, 0)
    return jnp.where(sub == 2, c - _hi(c), jnp.where(sub < 2, c, 0.0)).astype(bf16)


def _rows(b):
    return slice(b * RB, (b + 1) * RB)


def _cols(s):
    return slice(s * L, (s + 1) * L)


def _dot(a, b):
    return jnp.dot(a, b, preferred_element_type=f32)


def _kernel(x_hbm, wqkv_hbm, wo_hbm, w1_hbm, w2_hbm, w3_hbm, w4t_hbm, out_hbm,
            x_v, wqkv_v, wo_v, w1_v, w2_v, w3_v, w4t_v,
            wqkvt, wot, w1t, w2t, w3t, tmp32, tmpq,
            q_s, kp, vp, h_s, h1_s, hx_s, out_v, z_a, z_b, sems):
    ng = len(_GROUPS)
    ends = {f"x{p}": (x_hbm.at[:, j0 * C:j1 * C], x_v[p].at[0:D, :]) for p, (j0, j1) in enumerate(_XP)}
    for p, nm in enumerate(("wq", "wk", "wv")):
        ends[nm] = (wqkv_hbm.at[:, _QCOLS[p][0]:_QCOLS[p][1]], wqkv_v[p])
    ends.update(wo=(wo_hbm, wo_v), w1=(w1_hbm, w1_v), w2=(w2_hbm, w2_v), w3=(w3_hbm, w3_v),
                w4=(w4t_hbm, w4t_v), z=(z_a, z_b))
    groups = [[pltpu.make_async_copy(*ends[nm], sems.at[i]) for nm in spec.split()]
              for i, spec in enumerate(_GROUPS)]
    c_out = []
    st = {}
    lane1 = lax.broadcasted_iota(i32, (8, L), 1)

    def xloc(j, s=None):
        p = [p for p, (j0, j1) in enumerate(_XP) if j0 <= j < j1][0]
        c0 = (j - _XP[p][0]) * C
        return x_v[p], (slice(c0, c0 + C) if s is None else slice(c0 + s * L, c0 + (s + 1) * L))

    def gate_bits(gate):
        return pltpu.bitcast(gate, i32) & st["zvec"]

    def gated(p, gate):
        if gate is None:
            return p
        r, c = p.shape
        gz = pltpu.bitcast(gate_bits(gate), u32)
        if c < L:
            gz = gz[:, 0:c]
        elif c > L:
            gz = jnp.concatenate([gz] * (c // L), axis=1)
        return p | jnp.broadcast_to(gz[None], (r // 8, 8, c)).reshape(r, c)

    def tied(c, res):
        t = pltpu.bitcast(pltpu.bitcast(jnp.broadcast_to(c, (8, L)), i32) | gate_bits(res), f32)
        return jnp.broadcast_to(t[None], (RB // 8, 8, L)).reshape(RB, L)

    def note(name, res):
        st.setdefault(("res", name), []).extend(
            (res, r, s) for s in range(SUB) for r in range(res.shape[0] // 8))

    def pick_gates(spec, n):
        if not spec:
            return [None] * n
        tl = []
        for item in spec.split():
            nm, _, lim = item.partition(":")
            flat = st["res", nm]
            if lim:
                lo, hi = lim.split("-")
                flat = flat[len(flat) * int(lo) // 100:len(flat) * int(hi) // 100]
            tl += flat
        out = []
        for i in range(n):
            res, r, s = tl[(i * len(tl)) // n]
            out.append(res[r * 8:(r + 1) * 8, _cols(s)])
        return out

    lane_a = lax.broadcasted_iota(i32, (DB * 8, L), 1)

    def windows(ref, g, b, gate, done):
        rs = slice(b * DB * 8, (b + 1) * DB * 8)
        cur, prev = ref[g + 1, rs, :], ref[g, rs, :]
        if done is not None:
            gate = pltpu.bitcast(pltpu.bitcast(gate, i32) | pltpu.bitcast(done, i32), f32)
        prev = gated(prev, gate)
        for w in range(W):
            r = pltpu.roll(jnp.where(lane_a < L - DIL * w, cur, prev), DIL * w, 1) if w else cur
            t = _f32(r).reshape(DB, 2, 8, L)
            yield w, [t[:, 0], t[:, 1]]

    def att_qk(g, gates):
        lg = [[None] * W, [None] * W]
        hist = []
        for b in range(NBK):
            qb = q_s[g, b * DB * H:(b + 1) * DB * H, :].reshape(DB, 2, 8, L)
            for w, ks in windows(kp, g, b, gates[b], hist[b - 2] if b >= 2 else None):
                for i in range(2):
                    pr = jnp.sum(qb[:, i] * ks[i], axis=0)
                    lg[i][w] = pr if lg[i][w] is None else lg[i][w] + pr
            hist.append(lg[0][W - 1] + lg[1][W - 1] + lg[0][1])
        rq = st["rx", g] * (DH ** -0.5)
        a = []
        for i in range(2):
            sc = [t * rq for t in lg[i]]
            if g == 0:
                sc = [jnp.where(lane1 >= DIL * w, sc[w], -1e9) for w in range(W)]
            m = functools.reduce(jnp.maximum, sc)
            p = [jnp.exp(s_ - m) for s_ in sc]
            r = 1.0 / functools.reduce(jnp.add, p)
            a.append([p_ * r for p_ in p])
        st["att", g] = a

    def att_pv(g, gates):
        a = st["att", g]
        ob = []
        for b in range(NBK):
            o = [None, None]
            done = ob[b - 2][0:8] + ob[b - 2][DB * H - 8:] if b >= 2 else None
            for w, vs in windows(vp, g, b, gates[b], done):
                for i in range(2):
                    t = a[i][w][None] * vs[i]
                    o[i] = t if o[i] is None else o[i] + t
            ob.append(jnp.stack(o, axis=1).reshape(DB * H, L))
        st["o", g] = jnp.concatenate(ob, axis=0)

    def t_a(j, spec):
        gates = pick_gates(spec, SUB * 2 * NBK)
        for s in range(SUB):
            att_qk(j * SUB + s, gates[2 * s * NBK:(2 * s + 1) * NBK])
            att_pv(j * SUB + s, gates[(2 * s + 1) * NBK:(2 * s + 2) * NBK])

    def t_c(g, spec):
        att_qk(g, pick_gates(spec, NBK))

    def t_d(g, spec):
        att_pv(g, pick_gates(spec, NBK))

    def cat(key, j, rs=slice(None)):
        return jnp.concatenate([st[key, j * SUB + s][rs] for s in range(SUB)], axis=1).astype(bf16)

    def t_l(j, spec=None):
        gates = pick_gates(spec, SUB * NB)
        for s in range(SUB):
            xr, cs = xloc(j, s)
            a1 = a2 = None
            for b in range(NB):
                x = _f32(gated(_pk(xr[_rows(b), cs]), gates[s * NB + b]))
                a1 = x if a1 is None else a1 + x
                a2 = x * x if a2 is None else a2 + x * x
            m, v = _stats(a1, a2)
            st["rx", j * SUB + s] = lax.rsqrt(v + EPS)
            xr[D:DA, cs] = _mean_rows(m).astype(bf16)

    def qkv_epi(j, part, res):
        for s in range(SUB):
            g = j * SUB + s
            if part == 0:
                q_s[g] = res[:, _cols(s)]
            else:
                dst = kp if part == 1 else vp
                dst[g + 1] = _pk((res[:, _cols(s)] * st["rx", g]).astype(bf16))

    def t_Q(j):
        xr, cs = xloc(j)
        qkv = _dot(_up(wqkvt[...]), xr[:, cs])
        note(f"Q{j}", qkv)
        for p in range(3):
            qkv_epi(j, p, qkv[p * D:(p + 1) * D])

    def t_part(p, j):
        xr, cs = xloc(j)
        res = _dot(_up(wqkvt[p * D // 2:(p + 1) * D // 2, :]), xr[:, cs])
        note("qkv"[p] + str(j), res)
        qkv_epi(j, p, res)

    def t_O(j):
        ao = _dot(_up(wot[...]), cat("o", j))
        note(f"O{j}", ao)
        for s in range(SUB):
            g = j * SUB + s
            xr, cs = xloc(j, s)
            a1 = a2 = None
            hb = []
            done = None
            for b in range(NB):
                h = _f32(gated(_pk(xr[_rows(b), cs]), done)) + ao[_rows(b), _cols(s)]
                h_s[g, _rows(b), :] = h
                hb.append(h)
                a1 = h if a1 is None else a1 + h
                a2 = h * h if a2 is None else a2 + h * h
                done = jnp.sum((a1 + a2).reshape(RB // 8, 8, L), axis=0)
            m, v = _stats(a1, a2)
            r = lax.rsqrt(v + EPS)
            r2 = lax.rsqrt(v * r * r + EPS)
            st["h", g] = (m, r, _gelu_coef(r * r2))
            st["hb", g] = jnp.concatenate(hb + [_mean_rows(m)], axis=0)

    def t_M(j):
        a1 = _dot(_up(w1t[...]), cat("hb", j))
        note(f"M{j}", a1)
        for s in range(SUB):
            g = j * SUB + s
            ca, cb, ch = st["h", g][2]
            h1 = []
            for b in range(NB):
                y = a1[_rows(b), _cols(s)]
                hy = y * ch
                h1.append(hy + hy * jnp.tanh(y * (ca + cb * (y * y))))
            h1_s[g + 1] = _pk(jnp.concatenate(h1, axis=0).astype(bf16))

    grp = D // 8
    lane_g = lax.broadcasted_iota(i32, (grp, L), 1)

    def t_s(j):
        for s in range(SUB):
            g = j * SUB + s + 1
            parts = []
            for gi, sh in enumerate((1, -1, 2, -2)):
                gs = slice(gi * grp, (gi + 1) * grp)
                if sh > 0:
                    r = pltpu.roll(jnp.where(lane_g < L - sh, h1_s[g, gs, :], h1_s[g - 1, gs, :]), sh, 1)
                else:
                    r = pltpu.roll(jnp.where(lane_g >= -sh, h1_s[g, gs, :], h1_s[g + 1, gs, :]), L + sh, 1)
                parts.append(r)
            st["hsh", g - 1] = _up(jnp.concatenate(parts, axis=0))

    def t_P(j):
        hs = _dot(_up(w2t[...]), cat("hsh", j))
        note(f"P{j}", hs)
        for s in range(SUB):
            g = j * SUB + s
            m, r, _ = st["h", g]
            a1 = a2 = None
            xb = []
            for b in range(NB):
                h = h_s[g, _rows(b), :]
                x1 = (h - (tied(m, done) if b else m)) * r + hs[_rows(b), _cols(s)]
                hx_s[g, _rows(b), :] = h + x1
                xb.append(x1)
                a1 = x1 if a1 is None else a1 + x1
                a2 = x1 * x1 if a2 is None else a2 + x1 * x1
                done = jnp.sum((a1 + a2).reshape(RB // 8, 8, L), axis=0)
            m3, v3 = _stats(a1, a2)
            st["x", g] = _gelu_coef(lax.rsqrt(v3 + EPS))
            st["xb", g] = jnp.concatenate(xb + [_mean_rows(m3)], axis=0)

    def t_U(j):
        a3 = _dot(_up(w3t[...]), cat("xb", j))
        note(f"U{j}", a3)
        for s in range(SUB):
            ca, cb, _ = st["x", j * SUB + s]
            gb = []
            for b in range(F // RB):
                y = a3[_rows(b), _cols(s)]
                gb.append(y * (1.0 + jnp.tanh(y * (ca + cb * (y * y)))))
            st["g", j * SUB + s] = jnp.concatenate(gb, axis=0)

    def t_V(j):
        pieces = _LAST if j == NC - 1 else ((0, NB),)
        gj = {c: cat("g", j, slice(c, min(c + 512, F))) for c in range(0, F, 512)}
        for pi, (b0, b1) in enumerate(pieces):
            h2 = None
            for c in range(0, F, 512):
                e = min(c + 512, F)
                t = _dot(w4t_v[b0 * RB:b1 * RB, c:e], gj[c])
                note(f"V{j}", t)
                h2 = t if h2 is None else h2 + t
            for s in range(SUB):
                g = j * SUB + s
                ov = out_v[g + pi * SUB]
                ch = st["x", g][2]
                ov[...] = (hx_s[g, b0 * RB:b1 * RB, :] + h2[:, _cols(s)] * ch).astype(bf16)
                cp = pltpu.make_async_copy(ov, out_hbm.at[b0 * RB:b1 * RB, _cols(g)], sems.at[ng])
                cp.start()
                c_out.append(cp)

    def t_W(i):
        if i == 0:
            z_a[...] = jnp.zeros((8, L), i32)
            for group in groups:
                for c in group:
                    c.start()
            kp[0] = jnp.zeros((D // 2, L), u32)
            vp[0] = jnp.zeros((D // 2, L), u32)
            h1_s[0] = jnp.zeros((D // 2, L), u32)
            h1_s[NT + 1] = jnp.zeros((D // 2, L), u32)
        for c in groups[i]:
            c.wait()
        if i == 1:
            st["zvec"] = z_b[...]

    def t_Xpart(p):
        c0, c1 = _QCOLS[p]
        blk = [_pk(wqkv_v[p][b * 16:(b + 1) * 16, :]) for b in range(D // 16)]
        src = jnp.concatenate([_up(p_) for p_ in blk] + [_colsum_rows(blk)], axis=0).T.astype(f32)
        for c4 in range(4):
            wd = min(L, DA - c4 * L)
            tmpq[c4, c0:c1, 0:wd] = src[:, c4 * L:c4 * L + wd]
        for d in range(DH):
            for c4 in range(4):
                wd = min(L, DA - c4 * L)
                wqkvt[(p * D + d * H) // 2:(p * D + (d + 1) * H) // 2, c4 * L:c4 * L + wd] = (
                    _pk(tmpq[c4, pl.ds(p * D + d, H, stride=DH), 0:wd].astype(bf16)))

    def t_Xo(spec):
        gates = pick_gates(spec, 8)
        for c4 in range(4):
            wd = min(L, D - c4 * L)
            cs = slice(c4 * L, c4 * L + wd)
            for hf in range(2):
                p = gated(_pk(wo_v[hf * 224:(hf + 1) * 224, cs]), gates[c4 * 2 + hf])
                tmp32[c4, hf * 224:(hf + 1) * 224, 0:wd] = _f32(p)
            t = jnp.concatenate([tmp32[c4, pl.ds(d, H, stride=DH), 0:wd].astype(bf16) for d in range(DH)], axis=0)
            wot[c4 * L // 2:(c4 * L + wd) // 2, :] = _pk(t.T)

    def xpose_w(w_v, dst, n, xw, aug, spec):
        nb = -(-n // xw)
        gates = pick_gates(spec, nb * 4)
        for c in range(nb):
            c0, c1 = c * xw, min((c + 1) * xw, n)
            blk = [gated(_pk(w_v[b * 16:(b + 1) * 16, c0:c1]), gates[c * 4 + b // 7]) for b in range(D // 16)]
            t = jnp.concatenate([_up(p_) for p_ in blk] + ([_colsum_rows(blk)] if aug else []), axis=0)
            dst[c0 // 2:c1 // 2, :] = _pk(t.T)

    part = functools.partial
    once = dict(Xq=part(t_Xpart, 0), Xk=part(t_Xpart, 1), Xv=part(t_Xpart, 2), Xo=t_Xo,
                X1=part(xpose_w, w1_v, w1t, D, L, True), X2=part(xpose_w, w2_v, w2t, D, L, False),
                X3=part(xpose_w, w3_v, w3t, F, 256, True))
    per = dict(a=t_a, c=t_c, d=t_d, l=t_l, Q=t_Q, O=t_O, M=t_M, s=t_s, P=t_P, U=t_U, V=t_V, W=t_W,
               q=part(t_part, 0), k=part(t_part, 1), v=part(t_part, 2))
    for task in _ORDER:
        name, extra = (task[0], task[1:]) if isinstance(task, tuple) else (task, ())
        if name in once:
            once[name](*extra)
        else:
            per[name[0]](int(name[1:]), *extra)
    for c in c_out:
        c.wait()


@jax.jit
def pallas_sequential_preLN__sliding_local_dilated__mixer_s_mlp__prompt_kernel(
    A_x: jax.Array,
    A_wqkv: jax.Array,
    A_wo: jax.Array,
    B_x: jax.Array,
    B_w1: jax.Array,
    B_w2: jax.Array,
    B_w3: jax.Array,
    B_w4: jax.Array,
):
    del B_x
    hbm = pl.BlockSpec(memory_space=pl.ANY)
    V = pltpu.VMEM
    out_t = pl.pallas_call(
        _kernel,
        in_specs=[hbm] * 7,
        out_specs=hbm,
        out_shape=jax.ShapeDtypeStruct((D, S), bf16),
        scratch_shapes=[
            [V((DA, (j1 - j0) * C), bf16) for j0, j1 in _XP],
            [V((D, c1 - c0), bf16) for c0, c1 in _QCOLS],
            V((D, D), bf16), V((D, D), bf16),
            V((D, D), bf16), V((D, F), bf16), V((D, F), bf16),
            V((3 * D // 2, DA), u32), V((D // 2, D), u32), V((D // 2, DA), u32),
            V((D // 2, D), u32), V((F // 2, DA), u32),
            V((4, D, L), f32), V((4, 3 * D, L), f32),
            V((NT, D, L), f32), V((NT + 1, D // 2, L), u32), V((NT + 1, D // 2, L), u32),
            V((NT, D, L), f32), V((NT + 2, D // 2, L), u32), V((NT, D, L), f32),
            [V((D, L), bf16)] * (NT - SUB)
            + [V(((b1 - b0) * RB, L), bf16) for b0, b1 in _LAST for _ in range(SUB)],
            V((8, L), i32), V((8, L), i32),
            pltpu.SemaphoreType.DMA((len(_GROUPS) + 1,)),
        ],
        compiler_params=pltpu.CompilerParams(
            vmem_limit_bytes=100 * 1024 * 1024, disable_semaphore_checks=True),
    )(A_x.reshape(S, D).T, A_wqkv, A_wo, B_w1, B_w2, B_w3, B_w4.T)
    return out_t.T.reshape(1, S, D)
```
